```python
import jax
import jax.numpy as jnp

def _softmax(x, axis=-1):
    return jax.nn.softmax(x, axis=axis)
def _gelu(x):
    return jax.nn.gelu(x, approximate=True)
def _silu(x):
    return jax.nn.silu(x)
def _sigmoid(x):
    return jax.nn.sigmoid(x)
def _layernorm(x, axis=-1, eps=1e-5):
    m = jnp.mean(x, axis=axis, keepdims=True)
    v = jnp.var(x, axis=axis, keepdims=True)
    return (x - m) / jnp.sqrt(v + eps)
def _scatter_add(tgt, idx, src, axis=0):
    return tgt.at[idx].add(src)
def _segment_sum(src, seg, n):
    return jax.ops.segment_sum(src, seg, n)
class _Rng:
    def __init__(self, key):
        self._k = key
    def _next(self):
        self._k, sub = jax.random.split(self._k)
        return sub
    def normal(self, shape):
        return jax.random.normal(self._next(), shape, dtype=jnp.bfloat16)
    def randint(self, lo, hi, shape):
        return jax.random.randint(self._next(), shape, lo, hi, dtype=jnp.int32)
    def uniform(self, shape, lo=0.0, hi=1.0):
        return jax.random.uniform(self._next(), shape, jnp.bfloat16, lo, hi)
    def permutation(self, n):
        return jax.random.permutation(self._next(), n)


kernel_name = 'recurrent_scan__compressed_kv_cla__dense_activation_gelu__decode'

def setup_inputs():
    _rng = _Rng(jax.random.key(int.from_bytes(__import__("os").urandom(4), "little")))
    _w = (lambda a: (lambda t: t.astype(jnp.bfloat16) if jnp.issubdtype(t.dtype, jnp.floating) else t)(jnp.asarray(a)))
    def _A_setup():
        B, H, Sq, Sk, D, M = 2, 32, 1, 16384, 128, 512
        Dc = 4 * D
        return {
            "x": _w((lambda *s: _rng.normal(s) * 0.05)(B, Sq, M)),
            "c_kv": _w((lambda *s: _rng.normal(s) * 0.05)(B, Sk, Dc)),
            "w_q": _w((lambda *s: _rng.normal(s) * 0.05)(M, H, D) * (M ** -0.5)),
            "w_uk": _w((lambda *s: _rng.normal(s) * 0.05)(Dc, H, D) * (Dc ** -0.5)),
            "w_uv": _w((lambda *s: _rng.normal(s) * 0.05)(Dc, H, D) * (Dc ** -0.5)),
            "w_o": _w((lambda *s: _rng.normal(s) * 0.05)(H, D, M) * ((H * D) ** -0.5)),
        }
    _A_in = _A_setup()

    def _B_setup():
        B, S, D, F = 2, 1, 512, 1792
        return {
            "x": _w((lambda *s: _rng.normal(s) * 0.05)(B, S, D)),
            "w1": _w((lambda *s: _rng.normal(s) * 0.05)(D, F) * (D ** -0.5)),
            "b1": _w((lambda *s: _rng.normal(s) * 0.05)(F) * 0.01),
            "w2": _w((lambda *s: _rng.normal(s) * 0.05)(F, D) * (F ** -0.5)),
            "b2": _w((lambda *s: _rng.normal(s) * 0.05)(D) * 0.01),
        }
    _B_in = _B_setup()

    return {
        "A_x": _A_in["x"],
        "A_c_kv": _A_in["c_kv"],
        "A_w_q": _A_in["w_q"],
        "A_w_uk": _A_in["w_uk"],
        "A_w_uv": _A_in["w_uv"],
        "A_w_o": _A_in["w_o"],
        "B_x": _B_in["x"],
        "B_w1": _B_in["w1"],
        "B_b1": _B_in["b1"],
        "B_w2": _B_in["w2"],
        "B_b2": _B_in["b2"],
    }

def reference(A_x, A_c_kv, A_w_q, A_w_uk, A_w_uv, A_w_o, B_x, B_w1, B_b1, B_w2, B_b2):
    def _A_ref(x, c_kv, w_q, w_uk, w_uv, w_o):
        B, Sq, M = x.shape[0], x.shape[1], x.shape[2]
        Sk = c_kv.shape[1]
        H, D = w_q.shape[1], w_q.shape[2]
        q = jnp.einsum("bqm,mhd->bhqd", x, w_q)
        k = jnp.einsum("bkc,chd->bhkd", c_kv, w_uk)
        v = jnp.einsum("bkc,chd->bhkd", c_kv, w_uv)
        scores = jnp.einsum("bhqd,bhkd->bhqk", q, k) * (D ** -0.5)
        off = Sk - Sq
        qi = jnp.arange(Sq)[:, None]
        kj = jnp.arange(Sk)[None, :]
        cmask = kj <= (qi + off)
        scores = jnp.where(cmask[None, None], scores, -1e9)
        p = _softmax(scores, axis=-1)
        ctx = jnp.einsum("bhqk,bhkd->bhqd", p, v)
        return jnp.einsum("bhqd,hdm->bqm", ctx, w_o)

    def _B_ref(x, w1, b1, w2, b2):
        h = jnp.einsum("bsd,df->bsf", x, w1) + b1
        h = _gelu(h)
        return jnp.einsum("bsf,fd->bsd", h, w2) + b2

    x = A_x
    xn = _layernorm(x, axis=-1)
    s = _A_ref(xn, A_c_kv, A_w_q, A_w_uk, A_w_uv, A_w_o)
    g = _silu(_B_ref(xn, B_w1, B_b1, B_w2, B_b2))
    return x + s * g
```

```python
import contextlib
import jax
import jax.numpy as jnp
from jax import lax
import jax.experimental.pallas as pl
import jax.experimental.pallas.tpu as pltpu

F32 = jnp.float32
BF16 = jnp.bfloat16

B, H, SK, D, M, DC, F = 2, 32, 16384, 128, 512, 512, 1792
LOG2E = 1.4426950408889634
NT = (((1,), (1,)), ((), ()))

C_VIEW = (8, 4, 64, 16, DC)
W_VIEW = (4, 64, 2, H, D)
O_VIEW = (4, 2, 512, M)
W1_VIEW = (2, 32, 8, F)
W2_VIEW = (2, 112, 8, M)
W1_CUTS = ((0, 512), (512, 512), (1024, 384), (1408, 384))
LATE = (3, 11, 19, 7, 15, 23, 27, 29)


def _loop(lo, hi, body):
    lax.fori_loop(lo, hi, lambda i, _: body(i), None)


def _iota(shape, axis):
    return lax.broadcasted_iota(jnp.int32, shape, axis)


def _rows8(v):
    return jnp.concatenate([v[:, j * 128:(j + 1) * 128] for j in range(M // 128)], axis=0)


def make(TR=False, LAST=(16, 16), I4=(24, 40, 52, 68, 96), DL=10, QS=14, NOCOMP=False, LS=(0, 2, 4, 8, 12, 16, 22, 28), LX=(19, 25, 31),
         VS=28, M4=(3, 3), TAIL=(16,) * 32, LAG=28, STEPS=(16, 48, 64, 64, 64, 128), PS=((0, 1), (2,))):
    mains = [(0, M4[h], h, j * 16, 16) for j in range(32) for h in range(2)]
    t0 = 512 - sum(TAIL)
    mains += [(3, 1, 1, t0 + sum(TAIL[:i]), n) for i, n in enumerate(TAIL)]
    sides = sorted([((p + 4) / t0, 1, p) for p in range(0, t0, 8)] + [((p + 4) / 512, 0, p) for p in range(0, 512, 8) if M4[0] == 3])
    sides = [(3, 1, h, p, 8) for _, h, p in sides]
    NV = VS * 8 - 192
    assert NV + len(sides) == len(mains) == I4[-1], (NV, len(sides), len(mains))
    when = {d: i for i, d in enumerate(mains)}
    when.update({d: NV + i - LAG + 0.5 for i, d in enumerate(sides)})
    done = {}
    for (a, n, h, r, m), t in when.items():
        for u in range(a, a + n):
            done[8 * u + 4 * h + r // 128] = max(t, done.get(8 * u + 4 * h + r // 128, -99))
    group = {hd: max(0, int(t) // 16) for hd, t in done.items()}
    NM = PS[-1][-1] + 1
    vpu = sorted(hd for hd in group if group[hd] >= NM)
    late = sorted((d for d in when if 8 * d[0] + 4 * d[2] + d[3] // 128 in vpu), key=when.get)
    steps = [[]]
    for d in late[::-1]:
        if sum(e[1] * e[4] for e in steps[0]) >= STEPS[min(len(steps), len(STEPS)) - 1]:
            steps.insert(0, [])
        steps[0].insert(0, d)
    sem_of = {d: group[8 * d[0] + 4 * d[2] + d[3] // 128] for d in when}
    sem_of.update({d: NM + i for i, st in enumerate(steps) for d in st})

    def scope(name):
        return jax.named_scope('@' + name) if TR else contextlib.nullcontext()

    def kernel(x_hbm, c_hbm, wq_hbm, wuk_hbm, wuv_hbm, wo_hbm, w1_hbm, b1_hbm, w2_hbm, b2_hbm,
               o_hbm,
               x_buf, b1_buf, b2_buf, c_buf, wq_buf, wuk_buf, wuv_buf, wo_buf, w1_buf, w2_buf,
               xs, t8, qa_ref, acc_ref, m_ref, l_ref, e_buf, mul_ref, g_ref, o_buf,
               sem_w, sem_c, sem_o, sem_small):
        def main(src, dst, sem):
            pltpu.make_async_copy(src, dst, sem).start(priority=1)

        def side(src, dst, sem):
            pltpu.make_async_copy(src, dst, sem).start(priority=0)

        def wait_filled(buf, sem, name=''):
            with scope(name):
                pltpu.make_async_copy(buf, buf, sem).wait()

        def c_sem(b, e):
            if b == 0:
                return sem_c.at[e >> 5]
            k = 8 + (e >> 5)
            for i in range(1, len(LAST)):
                k = k + (e >= 256 - sum(LAST[i:])).astype(jnp.int32)
            return sem_c.at[k]

        def side_w2(e):
            side(w2_hbm.at[e & 1, e >> 1], w2_buf.at[e & 1, e >> 1], sem_w.at[4])

        def side_v(e):
            a, j, r = (e & 1) + ((e >> 3) & 2), 64 - VS + (e >> 5) * 4 + ((e >> 2) & 3), (e >> 1) & 1
            side(wuv_hbm.at[a, j, r], wuv_buf.at[a, j, r], sem_w.at[2])

        first = ((wuv_hbm, wuv_buf, 2), (wuk_hbm, wuk_buf, 1), (wq_hbm, wq_buf, 0))

        def issue1(lo, hi, arrays, e0):
            def body(j):
                e = e0 + j * (len(arrays) + 1)
                for i, (hbm, buf, k) in enumerate(arrays):
                    main(hbm.at[:, j], buf.at[:, j], sem_w.at[k])
                    side_w2(e + i)
                main(c_hbm.at[0, :, j], c_buf.at[0, j], c_sem(0, j))
                side_w2(e + len(arrays))
            _loop(lo, hi, body)

        def issue2(lo, hi):
            def body(j):
                for i in range(4):
                    b, e = (0, 64 + 3 * j + i) if i < 3 else (1, j)
                    main(c_hbm.at[1 + i, :, j], c_buf.at[b, e], c_sem(b, e))
                    cols = pl.ds(*W1_CUTS[i])
                    a, r = (j + i) & 1, j >> 1
                    side(w1_hbm.at[a, r, :, cols], w1_buf.at[a, r, :, cols], sem_w.at[3])
            with scope('i2'):
                _loop(lo, hi, body)

        def issue3(lo, hi):
            def body(j):
                for i in range(3):
                    e = 3 * j + i
                    main(c_hbm.at[5 + i, :, j], c_buf.at[1, 64 + e], c_sem(1, 64 + e))
                    side_v(e)
            with scope('i3'):
                _loop(lo, hi, body)

        def copy_o(go, d):
            a, n, h, r, m = d
            at = (a if n == 1 else pl.ds(a, n), h, pl.ds(r, m))
            go(wo_hbm.at[at], wo_buf.at[at], sem_o.at[sem_of[d]])

        def issue4(lo, hi):
            for i in range(lo, hi):
                copy_o(main, mains[i])
                if i < NV:
                    side_v(192 + i)
                else:
                    copy_o(side, sides[i - NV])

        def fenced4(k):
            with scope('i4'):
                _loop(0, one, lambda _: issue4(I4[k], I4[k + 1]))

        x_copy = pltpu.make_async_copy(x_hbm, x_buf, sem_small.at[0])
        b1_copy = pltpu.make_async_copy(b1_hbm, b1_buf, sem_small.at[1])
        b2_copy = pltpu.make_async_copy(b2_hbm, b2_buf, sem_small.at[2])

        small = [x_copy, b1_copy, b2_copy]
        for j in range(2):
            for i in range(16):
                a = i % 4
                if i < 12:
                    hbm, buf, k = first[i // 4]
                    main(hbm.at[a, j], buf.at[a, j], sem_w.at[k])
                else:
                    main(c_hbm.at[0, a, j], c_buf.at[0, j, a], c_sem(0, j))
                t = j * 16 + i
                if t in LS[:2 * (VS - 24)]:
                    e = LS.index(t)
                    cols = pl.ds(e % 2 * 256, 256)
                    side(w2_hbm.at[e // 2 % 2, e // 4, :, cols], w2_buf.at[e // 2 % 2, e // 4, :, cols], sem_w.at[4])
                if t in LX:
                    small[LX.index(t)].start()
                if a % 2 == 0 and DL:
                    pl.delay(DL)
        issue1(2, 64 - VS, first, VS - 32)

        x_copy.wait()
        x = x_buf[...].astype(F32)
        xc = x - jnp.mean(x, axis=-1, keepdims=True)
        var = jnp.mean(xc * xc, axis=-1, keepdims=True)
        xn = (xc * lax.rsqrt(var + 1e-5)).astype(BF16)
        xf = xn.astype(F32)
        for b in range(B):
            for j in range(M // 128):
                cols = slice(j * 128, (j + 1) * 128)
                xs[b, cols, :] = jnp.broadcast_to(xf[b:b + 1, cols], (128, 128)).T
        col, row = _iota((128, 1024), 1), _iota((128, 1024), 0)
        e_buf[...] = (col >> 3 == row).astype(F32).astype(BF16)
        m_ref[...] = jnp.full((B * H, 128), -jnp.inf, F32)
        l_ref[...] = jnp.zeros((B * H, 128), F32)
        acc_ref[...] = jnp.zeros((B * H, DC), F32)
        issue1(64 - VS, 64, first[1:], 32)
        issue2(0, QS)

        wait_filled(wq_buf, sem_w.at[0], 'wq')

        def q_body(i, carry):
            pl.when((i & 15) == 15)(lambda: issue2(QS + (i >> 4) * 2, QS + (i >> 4) * 2 + 2))
            q0, q1 = carry
            for u in range(0 if NOCOMP else 8):
                m = pl.ds(i * 8 + u, 1)
                w = wq_buf[i >> 4, (i & 15) * 4 + u // 2, u % 2].astype(F32)
                q0 = q0 + xs[0, m, :] * w
                q1 = q1 + xs[1, m, :] * w
            return q0, q1

        q0, q1 = lax.fori_loop(0, 64, q_body, (jnp.zeros((H, D), F32), jnp.zeros((H, D), F32)))
        q = jnp.concatenate([q0, q1, jnp.zeros((128 - B * H, D), F32)], axis=0).astype(BF16)

        wait_filled(wuk_buf, sem_w.at[1], 'wuk')
        hgroup = (_iota((16, 8, 128), 2) % H) // 8

        def qa_body(i):
            for u in range(0 if NOCOMP else 8):
                w = wuk_buf[i, pl.ds(u * 8, 8)].reshape(16 * H, D)
                r = lax.dot_general(w, q, NT, preferred_element_type=F32).reshape(16, 4, 8, 128)
                v = jnp.where(hgroup == 0, r[:, 0],
                              jnp.where(hgroup == 1, r[:, 1], jnp.where(hgroup == 2, r[:, 2], r[:, 3])))
                t8[pl.ds(pl.multiple_of((i * 8 + u) * 128, 128), 128), :] = v.reshape(128, 128)
            issue2(QS + 8 + 2 * i, QS + 10 + 2 * i)

        _loop(0, 4, qa_body)
        sub = _iota((128, 128), 1) % 8
        for j in range(DC // 128):
            t = t8[pl.ds(j * 1024, 128, stride=8), :]
            for s in range(1, 8):
                t = jnp.where(sub == s, t8[pl.ds(j * 1024 + s, 128, stride=8), :], t)
            qa_ref[:, j * 128:(j + 1) * 128] = (t.T[:B * H] * (D ** -0.5 * LOG2E)).astype(BF16)

        def attend(b, e, n, sem):
            wait_filled(c_buf.at[b, pl.ds(e, n)], sem, 'c')
            if NOCOMP:
                return
            hrows = pl.ds(b * H if isinstance(b, int) else pl.multiple_of(b * H, H), H)
            c = c_buf[b, pl.ds(e, n)].reshape(n * 64, DC)
            sc = lax.dot_general(qa_ref[hrows, :], c, NT, preferred_element_type=F32)
            m_prev = m_ref[hrows, :]
            m_new = jnp.maximum(m_prev, jnp.max(sc, axis=1, keepdims=True))
            p = jnp.exp2(sc - m_new[:, :1])
            alpha = jnp.exp2(m_prev - m_new)
            l_ref[hrows, :] = alpha * l_ref[hrows, :] + jnp.sum(p, axis=1, keepdims=True)
            m_ref[hrows, :] = m_new
            pv = jnp.dot(p.astype(BF16), c, preferred_element_type=F32)
            acc_ref[hrows, :] = acc_ref[hrows, :] * alpha[:, :1] + pv

        def gate():
            wait_filled(w1_buf, sem_w.at[3], 'w1')
            wait_filled(w2_buf, sem_w.at[4], 'w2')
            b1_copy.wait()
            b2_copy.wait()
            hid = jnp.dot(xn, w1_buf[...].reshape(M, F), preferred_element_type=F32)
            hid = jax.nn.gelu(hid + b1_buf[...].astype(F32).reshape(1, F), approximate=True).astype(BF16)
            z = jnp.dot(hid, w2_buf[...].reshape(F, M), preferred_element_type=F32)
            z8 = _rows8(z + b2_buf[...].astype(F32).reshape(1, M))
            g_ref[0] = z8 * jax.nn.sigmoid(z8)
            g_ref[1] = _rows8(x)

        R0 = QS + 16

        def block(i):
            pl.when(i < 6)(lambda: issue2(R0 + i * (64 - R0) // 6, R0 + (i + 1) * (64 - R0) // 6))

            @pl.when(jnp.logical_and(i >= 6, i < 14))
            def _():
                issue3((i - 6) * 8, (i - 6) * 8 + 5)
                pl.when(i == 10)(gate)
                issue3((i - 6) * 8 + 5, (i - 6) * 8 + 8)
            pl.when(i == 14)(lambda: issue4(0, I4[0]))
            k = jnp.where(i == 7, 8, jnp.where(i == 8, 7, i))
            attend(k >> 3, (k & 7) * 32, 32, sem_c.at[k])

        one = lax.fori_loop(0, 15, lambda i, c: (block(i), (c + i) & 1)[1], 0)
        for i, n in enumerate(LAST):
            fenced4(i)
            attend(1, 256 - sum(LAST[i:]), n, sem_c.at[15 + i])

        fenced4(len(LAST))
        wait_filled(wuv_buf, sem_w.at[2], 'wuv')
        pc = acc_ref[...] / l_ref[...][:, :1]
        pc = jnp.concatenate([pc[b * H + g * 8:b * H + g * 8 + 8, j * 128:(j + 1) * 128]
                              for g in range(4) for j in range(4) for b in range(B)], axis=0).astype(BF16)
        rep = jnp.dot(pc, e_buf[...], preferred_element_type=F32)
        rep = jnp.where((col & 7) == (row & 7), rep.reshape(2, 128, 1024), 0.0).astype(BF16).reshape(4, 4, 16, 1024)
        ctx = []
        for g in range(4):
            a = jnp.concatenate([rep[g, j] for j in range(4)], axis=1)
            w = wuv_buf[:, :, :, g * 8:g * 8 + 8].reshape(DC * 8, D)
            ctx.append(jnp.dot(a, w, preferred_element_type=F32).astype(BF16).astype(F32))
        fenced4(len(LAST) + 1)

        sl16 = _iota((16, 128), 0) & 7

        def project(heads):
            lhs = jnp.concatenate([jnp.where(sl16 == h % 8, ctx[h // 8], 0.0) for h in heads], axis=1)
            rhs = jnp.concatenate([wo_buf[h // 8, h // 4 % 2, pl.ds(h % 4 * D, D)] for h in heads], axis=0)
            return jnp.dot(lhs.astype(BF16), rhs, preferred_element_type=F32)

        s = []
        for ks in PS:
            for k in ks:
                wait_filled(c_buf.at[0, pl.ds(0, 2 * sum(v == k for v in group.values()))], sem_o.at[k], 'o')
            if not s:
                for b in range(B):
                    for k, h in enumerate(vpu):
                        r = b * 8 + h % 8
                        mul_ref[b, k * D:(k + 1) * D] = jnp.broadcast_to(ctx[h // 8][r:r + 1], (128, 128)).T
            t = project([h for h in sorted(group) if group[h] in ks])
            s.append([[t[b * 8:b * 8 + 8, j * 128:(j + 1) * 128] for j in range(4)] for b in range(B)])

        part = [[sum((t[b][j] for t in s[1:]), s[0][b][j]) for j in range(4)] for b in range(B)]
        g8, x8 = g_ref[0], g_ref[1]
        sl = _iota((8, 128), 0)
        masks = {k: (sl & k) != 0 for k in (1, 2, 4)}
        for i, st in enumerate(steps):
            wait_filled(w2_buf.at[0, pl.ds(0, sum(d[1] * d[4] for d in st) // 8)], sem_o.at[NM + i], 'last')
            for a, n, h, r0, m in st:
                for u in range(a, a + n):
                    for r in range(r0, r0 + m, 8):
                        w = wo_buf[u, h, r:r + 8].astype(F32)
                        for b in range(B):
                            mul = mul_ref[b, pl.ds(vpu.index(8 * u + 4 * h + r // 128) * D + r % D, 8), :]
                            for j in range(M // 128):
                                part[b][j] = part[b][j] + w[:, j * 128:(j + 1) * 128] * mul

        def merge(lo, hi, k):
            m = masks[k]
            if k == 4:
                return jnp.where(m, hi, lo) + pltpu.roll(jnp.where(m, lo, hi), 4, 0)
            return jnp.where(m, hi, lo) + jnp.where(m, pltpu.roll(hi, k, 0), pltpu.roll(lo, 8 - k, 0))

        r4 = [[merge(part[b][j], part[b][j + 2], 4) for j in range(2)] for b in range(B)]
        r2 = [merge(r4[b][0], r4[b][1], 2) for b in range(B)]
        o_buf[...] = (x8 + g8 * merge(r2[0], r2[1], 1)).astype(BF16)
        o_copy = pltpu.make_async_copy(o_buf, o_hbm, sem_small.at[0])
        o_copy.start()
        o_copy.wait()

    def fn(A_x, A_c_kv, A_w_q, A_w_uk, A_w_uv, A_w_o, B_x, B_w1, B_b1, B_w2, B_b2):
        hbm = pl.BlockSpec(memory_space=pltpu.HBM)
        sems = pltpu.SemaphoreType.DMA
        out = pl.pallas_call(
            kernel,
            out_shape=jax.ShapeDtypeStruct((8, 128), BF16),
            in_specs=[hbm] * 10,
            out_specs=hbm,
            scratch_shapes=[
                pltpu.VMEM((B, M), BF16), pltpu.VMEM((F,), BF16), pltpu.VMEM((M,), BF16),
                pltpu.VMEM((B, 256, 4, 16, DC), BF16), pltpu.VMEM(W_VIEW, BF16), pltpu.VMEM(W_VIEW, BF16),
                pltpu.VMEM(W_VIEW, BF16), pltpu.VMEM(O_VIEW, BF16),
                pltpu.VMEM(W1_VIEW, BF16), pltpu.VMEM(W2_VIEW, BF16),
                pltpu.VMEM((B, M, 128), F32),
                pltpu.VMEM((DC * 8 + 8, 128), F32),
                pltpu.VMEM((B * H, DC), BF16), pltpu.VMEM((B * H, DC), F32),
                pltpu.VMEM((B * H, 128), F32), pltpu.VMEM((B * H, 128), F32),
                pltpu.VMEM((128, 1024), BF16),
                pltpu.VMEM((B, len(vpu) * D, 128), F32), pltpu.VMEM((2, 8, 128), F32),
                pltpu.VMEM((8, 128), BF16),
                sems((5,)), sems((15 + len(LAST),)), sems((NM + len(steps),)),
                sems((3,)),
            ],
            compiler_params=pltpu.CompilerParams(
                vmem_limit_bytes=100 * 1024 * 1024, disable_semaphore_checks=True, disable_bounds_checks=True),
        )(A_x.reshape(B, M), A_c_kv.reshape(C_VIEW), A_w_q.reshape(W_VIEW), A_w_uk.reshape(W_VIEW),
          A_w_uv.reshape(W_VIEW), A_w_o.reshape(O_VIEW), B_w1.reshape(W1_VIEW), B_b1, B_w2.reshape(W2_VIEW), B_b2)
        return out.reshape(M // 128, B, 128).transpose(1, 0, 2).reshape(B, 1, M)
    assert sum(LAST) == 32
    return fn


@jax.jit
def pallas_recurrent_scan__compressed_kv_cla__dense_activation_gelu__decode_kernel(
    A_x, A_c_kv, A_w_q, A_w_uk, A_w_uv, A_w_o, B_x, B_w1, B_b1, B_w2, B_b2,
):
    return make(DL=0, STEPS=(16,32,32,48,64,64,128))(A_x, A_c_kv, A_w_q, A_w_uk, A_w_uv, A_w_o, B_x, B_w1, B_b1, B_w2, B_b2)
```

```python
import contextlib
import jax
import jax.numpy as jnp
from jax import lax
import jax.experimental.pallas as pl
import jax.experimental.pallas.tpu as pltpu

F32 = jnp.float32
BF16 = jnp.bfloat16

B, H, SK, D, M, DC, F = 2, 32, 16384, 128, 512, 512, 1792
LOG2E = 1.4426950408889634
NT = (((1,), (1,)), ((), ()))

C_VIEW = (8, 4, 64, 16, DC)
W_VIEW = (4, 64, 2, H, D)
O_VIEW = (4, 8 * D, M)
W_QUADS = 192
S_UV, S_UK, S_Q, S_W1, S_W2, S_X, S_B1, S_B2, S_C = range(9)
S_O = S_C + 32


def _loop(lo, hi, body):
    lax.fori_loop(lo, hi, lambda i, _: body(i), None)


def _iota(shape, axis):
    return lax.broadcasted_iota(jnp.int32, shape, axis)


def _rows8(v):
    return jnp.concatenate([v[:, j * 128:(j + 1) * 128] for j in range(M // 128)], axis=0)


def make(TR=False, E1=10, E2=8, SH=0, TAIL=(16,) * 16 + (8,) * 16, LAG=26, STEPS=(8,) * 4 + (16,) * 8 + (32,), NOCOMP=False, NOTAIL=False, EA=(True, False, False), SM=30,
         AHEAD=57, CUT=(0.07, 0.15, 0.24, 0.33, 0.44, 0.57, 0.65, 0.71, 0.79, 0.87, 0.94, 1.0), FIN='0 1 h 2 g', SWAPS=(78, 500)):
    def ffn(t, h):
        out = []
        for k in range(8 + h, 0, -2):
            x = 3584 + SH - 512 * k + t % 32 * 16
            if 0 <= x < 1792 and -E2 <= t < 32 - E2:
                out.append(('w2', x))
            if 1792 <= x < 3584 and -E1 <= t < 32 - E1:
                r, c = divmod(x - 1792, 28)
                out.append(('w1', r, c, min(16, 28 - c)))
                if c > 12:
                    out.append(('w1', r + 1, 0, c - 12))
        return out

    C_END = 512 - 4 * max(E1, E2)
    first = [('o', 3, 1, 512 + sum(TAIL) + 8 * i, 8) for i in range(8)]
    quads = []
    for e in range(C_END, 512):
        if e % 2 == 0:
            quads.append(ffn(e // 4 - 128, e // 2 % 2))
        quads.append([('c', e, 1), ('c', e, 0)])
    for j in range(64):
        row = j // 2 * 16 + j % 2 * 512
        quads.append(ffn(j // 2, j % 2))
        quads.append([('o', 0, 3, row, 16), None if 512 <= row <= first[-1][3] else ('o', 3, 1, row, 16)])
    quads += [[('o', 3, 1, 512 + sum(TAIL[:i]), n), None] for i, n in enumerate(TAIL)]
    served = [(None, [('c', e, 0)]) for e in range(C_END - LAG, C_END)]
    for quad in quads:
        served += [(d, []) for d in quad[:-1]]
        served[-1][1].extend(d for d in quad[-1:] if d)
    ending = [x for (m, _), (_, s) in zip(served[LAG:], served) for x in [(m, 1)] + [(d, 0) for d in s]]
    assert not any(s for _, s in served[-LAG:])

    vpu = [h for h in range(H) if h % 4 == 3 or h >= 28]
    late = [d for d in first + [d for m, s in served[LAG:] for d in [m] + s] if d[0] == 'o' and 8 * d[1] + d[3] // D in vpu]
    steps = [[]]
    for d in late[::-1]:
        if sum(e[2] * e[4] for e in steps[0]) >= STEPS[min(len(steps), len(STEPS)) - 1]:
            steps.insert(0, [])
        steps[0].insert(0, d)
    step_of = {d: i for i, st in enumerate(steps) for d in st}
    IN_LOOP = (C_END - AHEAD) // 32
    cuts = [0] + [round(c * len(ending)) for c in CUT]

    def scope(name):
        return jax.named_scope('@' + name) if TR else contextlib.nullcontext()

    def kernel(x_hbm, c_hbm, wq_hbm, wuk_hbm, wuv_hbm, wo_hbm, w1_hbm, b1_hbm, w2_hbm, b2_hbm,
               o_hbm,
               x_buf, b1_buf, b2_buf, c_buf, wq_buf, wuk_buf, wuv_buf, wo_buf, w1_buf, w2_buf,
               xs, t8, qa_ref, acc_ref, m_ref, l_ref, e_buf, a_buf, ctx_ref, mul_ref, o_buf, sems):
        def wait_filled(buf, k, name=''):
            with scope(name):
                pltpu.make_async_copy(buf, buf, sems.at[k]).wait()

        runs = (3, pl.ds(0, 3))

        def fetch_w(j, i, queue):
            hbm, buf = ((wuv_hbm, wuv_buf), (wuk_hbm, wuk_buf), (wq_hbm, wq_buf))[i]
            pltpu.make_async_copy(hbm.at[runs[queue], j], buf.at[runs[queue], j], sems.at[i]).start(priority=queue)

        def fetch_c(e, queue):
            src = c_hbm.at[(e >> 8) * 4 + (e & 3), runs[queue], (e >> 2) & 63]
            pltpu.make_async_copy(src, c_buf.at[e, runs[queue]], sems.at[S_C + (e >> 4)]).start(priority=queue)

        def fetch(d, queue):
            if d[0] == 'c':
                return fetch_c(d[1], queue)
            if d[0] == 'w2':
                hbm, buf, at, k = w2_hbm, w2_buf, pl.ds(d[1], 16), S_W2
            elif d[0] == 'w1':
                hbm, buf, at, k = w1_hbm, w1_buf, (pl.ds(d[1] * 8, 8), pl.ds(d[2] * 64, d[3] * 64)), S_W1
            else:
                hbm, buf, at = wo_hbm, wo_buf, (runs[d[2] > 1], pl.ds(d[3], d[4]))
                k = S_O + (3 + step_of[d] if d in step_of else d[3] // D % 4)
            pltpu.make_async_copy(hbm.at[at], buf.at[at], sems.at[k]).start(priority=queue)

        def issue_w(lo, hi, early=False):
            def body(j):
                for i in range(3):
                    for queue in ((0, 1) if early else (1, 0)):
                        r, a = divmod(i - (1 - queue) * LAG, 3)
                        fetch_w(j + r, a, queue)
            _loop(lo, hi, body)

        def issue_c(lo, hi, early=False):
            def body(e):
                for queue in ((0, 1) if early else (1, 0)):
                    fetch_c(e - (1 - queue) * LAG, queue)
            with scope('ic'):
                _loop(lo, hi, body)

        done = [0]

        def issue_end():
            lo, hi = cuts[done[0]:done[0] + 2]
            done[0] += 1

            def body(_):
                for d, queue in ending[lo:hi]:
                    fetch(d, queue)
            with scope('ie'):
                _loop(0, one, body)

        x_copy = pltpu.make_async_copy(x_hbm, x_buf, sems.at[S_X])
        b1_copy = pltpu.make_async_copy(b1_hbm, b1_buf, sems.at[S_B1])
        b2_copy = pltpu.make_async_copy(b2_hbm, b2_buf, sems.at[S_B2])

        for i in range(27):
            fetch_w(*divmod(i, 3), 1)
            if i >= LAG:
                fetch_w(*divmod(i - LAG, 3), 0)
            elif i % 3 == 0 and i < 24:
                fetch(first[i // 3], 0)
            elif i == SM:
                for c in (x_copy, b2_copy, b1_copy):
                    c.start()
        issue_w(9, 20)
        if SM > 26:
            for c in (x_copy, b2_copy, b1_copy):
                c.start()
        issue_w(20, SWAPS[0] // 3, EA[0])

        x_copy.wait()
        x = x_buf[...].astype(F32)
        xc = x - jnp.mean(x, axis=-1, keepdims=True)
        var = jnp.mean(xc * xc, axis=-1, keepdims=True)
        xn = (xc * lax.rsqrt(var + 1e-5)).astype(BF16)
        xf = xn.astype(F32)
        for b in range(B):
            for j in range(M // 128):
                cols = slice(j * 128, (j + 1) * 128)
                xs[b, cols, :] = jnp.broadcast_to(xf[b:b + 1, cols], (128, 128)).T
        col, row = _iota((128, 1024), 1), _iota((128, 1024), 0)
        e_buf[...] = (col >> 3 == row).astype(F32).astype(BF16)
        m_ref[...] = jnp.full((B * H, 128), -jnp.inf, F32)
        l_ref[...] = jnp.zeros((B * H, 128), F32)
        acc_ref[...] = jnp.zeros((B * H, DC), F32)
        issue_w(SWAPS[0] // 3, 64)
        for e in range(LAG):
            fetch_c(e, 1)
            fetch_w(*divmod(W_QUADS - LAG + e, 3), 0)
        issue_c(LAG, AHEAD, EA[1])

        wait_filled(wq_buf, S_Q, 'wq')

        def q_body(i, carry):
            pl.when((i & 15) == 15)(lambda: issue_c(AHEAD + (i >> 4) * 10, AHEAD + (i >> 4) * 10 + 10))
            q0, q1 = carry
            for u in range(0 if NOCOMP else 8):
                m = pl.ds(i * 8 + u, 1)
                w = wq_buf[i >> 4, (i & 15) * 4 + u // 2, u % 2].astype(F32)
                q0 = q0 + xs[0, m, :] * w
                q1 = q1 + xs[1, m, :] * w
            return q0, q1

        q0, q1 = lax.fori_loop(0, 64, q_body, (jnp.zeros((H, D), F32), jnp.zeros((H, D), F32)))
        q = jnp.concatenate([q0, q1, jnp.zeros((128 - B * H, D), F32)], axis=0).astype(BF16)

        wait_filled(wuk_buf, S_UK, 'wuk')
        group = (_iota((16, 8, 128), 2) % H) // 8

        def qa_body(i):
            for u in range(0 if NOCOMP else 8):
                w = wuk_buf[i, pl.ds(u * 8, 8)].reshape(16 * H, D)
                r = lax.dot_general(w, q, NT, preferred_element_type=F32).reshape(16, 4, 8, 128)
                v = jnp.where(group == 0, r[:, 0],
                              jnp.where(group == 1, r[:, 1], jnp.where(group == 2, r[:, 2], r[:, 3])))
                t8[pl.ds(pl.multiple_of((i * 8 + u) * 128, 128), 128), :] = v.reshape(128, 128)
            issue_c(AHEAD + 40 + 13 * i, AHEAD + 53 + 13 * i)

        _loop(0, 4, qa_body)
        sub = _iota((128, 128), 1) % 8
        for j in range(DC // 128):
            t = t8[pl.ds(j * 1024, 128, stride=8), :]
            for s in range(1, 8):
                t = jnp.where(sub == s, t8[pl.ds(j * 1024 + s, 128, stride=8), :], t)
            qa_ref[:, j * 128:(j + 1) * 128] = (t.T[:B * H] * (D ** -0.5 * LOG2E)).astype(BF16)

        def attend(k, n):
            for i in range(n):
                wait_filled(c_buf.at[pl.ds((k + i) * 16, 16)], S_C + k + i, 'c')
            if NOCOMP:
                return
            hrows = pl.ds((k >> 4) * H if isinstance(k, int) else pl.multiple_of((k >> 4) * H, H), H)
            c = c_buf[pl.ds(k * 16, n * 16)].reshape(n * 1024, DC)
            sc = lax.dot_general(qa_ref[hrows, :], c, NT, preferred_element_type=F32)
            m_prev = m_ref[hrows, :]
            m_new = jnp.maximum(m_prev, jnp.max(sc, axis=1, keepdims=True))
            p = jnp.exp2(sc - m_new[:, :1])
            alpha = jnp.exp2(m_prev - m_new)
            l_ref[hrows, :] = alpha * l_ref[hrows, :] + jnp.sum(p, axis=1, keepdims=True)
            m_ref[hrows, :] = m_new
            pv = jnp.dot(p.astype(BF16), c, preferred_element_type=F32)
            acc_ref[hrows, :] = acc_ref[hrows, :] * alpha[:, :1] + pv

        def block(i, lo):
            hi = jnp.maximum(AHEAD + 100 + 22 * i, C_END - 32 * (IN_LOOP - i))
            issue_c(lo, hi)
            attend(2 * i, 2)
            return hi

        lo = lax.fori_loop(0, IN_LOOP, block, AHEAD + 92)
        issue_c(lo, C_END, EA[2])
        one = (lo > 0).astype(jnp.int32)
        attend(2 * IN_LOOP, 2)
        for k in range(2 * IN_LOOP + 2, 32):
            issue_end()
            attend(k, 1)

        issue_end()
        pc = acc_ref[...] / l_ref[...][:, :1]
        pc = jnp.concatenate([pc[b * H + g * 8:b * H + g * 8 + 8, j * 128:(j + 1) * 128]
                              for g in range(4) for j in range(4) for b in range(B)], axis=0).astype(BF16)
        rep = jnp.dot(pc, e_buf[...], preferred_element_type=F32).reshape(2, 128, 1024)
        a_buf[...] = jnp.where((col & 7) == (row & 7), rep, 0.0).astype(BF16).reshape(16, 16, 1024)
        issue_end()
        wait_filled(wuv_buf, S_UV, 'wuv')
        for g in range(4):
            a = jnp.concatenate([a_buf[4 * g + j] for j in range(4)], axis=1)
            w = wuv_buf[:, :, :, g * 8:g * 8 + 8].reshape(DC * 8, D)
            ctx_ref[g] = jnp.dot(a, w, preferred_element_type=F32).astype(BF16).astype(F32)
        issue_end()
        for b in range(B):
            for k, h in enumerate(vpu):
                mul_ref[b, k * D:(k + 1) * D] = jnp.broadcast_to(ctx_ref[h // 8, pl.ds(b * 8 + h % 8, 1)], (128, 128)).T

        sl16 = _iota((16, 128), 0) & 7
        part = [[None] * 4 for _ in range(B)]
        for what in FIN.split():
            if done[0] < len(CUT):
                issue_end()
            if what == 'h':
                wait_filled(w1_buf, S_W1, 'w1')
                b1_copy.wait()
                hid = jnp.dot(xn, w1_buf[...], preferred_element_type=F32)
                hid = jax.nn.gelu(hid + b1_buf[...].astype(F32).reshape(1, F), approximate=True).astype(BF16)
            elif what == 'g':
                wait_filled(w2_buf, S_W2, 'w2')
                b2_copy.wait()
                z = jnp.dot(hid, w2_buf[...], preferred_element_type=F32)
                z8 = _rows8(z + b2_buf[...].astype(F32).reshape(1, M))
                g8 = z8 * jax.nn.sigmoid(z8)
                x8 = _rows8(x)
            else:
                wait_filled(wo_buf.at[0, pl.ds(0, 7 * D)], S_O + int(what), 'o')
                heads = range(int(what), 28, 4)
                lhs = jnp.concatenate([jnp.where(sl16 == h % 8, ctx_ref[h // 8], 0.0) for h in heads], axis=1)
                rhs = jnp.concatenate([wo_buf[h // 8, pl.ds(h % 8 * D, D)] for h in heads], axis=0)
                s = jnp.dot(lhs.astype(BF16), rhs, preferred_element_type=F32)
                for b in range(B):
                    for j in range(4):
                        t = s[b * 8:b * 8 + 8, j * 128:(j + 1) * 128]
                        part[b][j] = t if part[b][j] is None else part[b][j] + t
        assert done[0] == len(CUT)

        sl = _iota((8, 128), 0)
        masks = {k: (sl & k) != 0 for k in (1, 2, 4)}
        for i, st in enumerate(steps):
            wait_filled(wo_buf.at[0, pl.ds(0, sum(d[2] * d[4] for d in st))], S_O + 3 + i, 'last')
            for _, a, n, r0, m in ([] if NOTAIL else st):
                for u in range(a, a + n):
                    for r in range(r0, r0 + m, 8):
                        w = wo_buf[u, r:r + 8].astype(F32)
                        for b in range(B):
                            mul = mul_ref[b, pl.ds(vpu.index(8 * u + r // D) * D + r % D, 8), :]
                            for j in range(M // 128):
                                part[b][j] = part[b][j] + w[:, j * 128:(j + 1) * 128] * mul

        def merge(lo, hi, k):
            m = masks[k]
            if k == 4:
                return jnp.where(m, hi, lo) + pltpu.roll(jnp.where(m, lo, hi), 4, 0)
            return jnp.where(m, hi, lo) + jnp.where(m, pltpu.roll(hi, k, 0), pltpu.roll(lo, 8 - k, 0))

        r4 = [[merge(part[b][j], part[b][j + 2], 4) for j in range(2)] for b in range(B)]
        r2 = [merge(r4[b][0], r4[b][1], 2) for b in range(B)]
        o_buf[...] = (x8 + g8 * merge(r2[0], r2[1], 1)).astype(BF16)
        o_copy = pltpu.make_async_copy(o_buf, o_hbm, sems.at[S_X])
        o_copy.start()
        o_copy.wait()

    def fn(A_x, A_c_kv, A_w_q, A_w_uk, A_w_uv, A_w_o, B_x, B_w1, B_b1, B_w2, B_b2):
        hbm = pl.BlockSpec(memory_space=pltpu.HBM)
        out = pl.pallas_call(
            kernel,
            out_shape=jax.ShapeDtypeStruct((8, 128), BF16),
            in_specs=[hbm] * 10,
            out_specs=hbm,
            scratch_shapes=[
                pltpu.VMEM((B, M), BF16), pltpu.VMEM((F,), BF16), pltpu.VMEM((M,), BF16),
                pltpu.VMEM((512, 4, 16, DC), BF16), pltpu.VMEM(W_VIEW, BF16), pltpu.VMEM(W_VIEW, BF16),
                pltpu.VMEM(W_VIEW, BF16), pltpu.VMEM(O_VIEW, BF16),
                pltpu.VMEM((M, F), BF16), pltpu.VMEM((F, M), BF16),
                pltpu.VMEM((B, M, 128), F32),
                pltpu.VMEM((DC * 8 + 8, 128), F32),
                pltpu.VMEM((B * H, DC), BF16), pltpu.VMEM((B * H, DC), F32),
                pltpu.VMEM((B * H, 128), F32), pltpu.VMEM((B * H, 128), F32),
                pltpu.VMEM((128, 1024), BF16), pltpu.VMEM((16, 16, 1024), BF16), pltpu.VMEM((4, 16, D), F32),
                pltpu.VMEM((B, len(vpu) * D, 128), F32), pltpu.VMEM((8, 128), BF16),
                pltpu.SemaphoreType.DMA((S_O + 3 + len(steps),)),
            ],
            compiler_params=pltpu.CompilerParams(
                vmem_limit_bytes=100 * 1024 * 1024, disable_semaphore_checks=True, disable_bounds_checks=True),
        )(A_x.reshape(B, M), A_c_kv.reshape(C_VIEW), A_w_q.reshape(W_VIEW), A_w_uk.reshape(W_VIEW),
          A_w_uv.reshape(W_VIEW), A_w_o.reshape(O_VIEW), B_w1, B_b1, B_w2, B_b2)
        return out.reshape(M // 128, B, 128).transpose(1, 0, 2).reshape(B, 1, M)
    return fn


@jax.jit
def pallas_recurrent_scan__compressed_kv_cla__dense_activation_gelu__decode_kernel(
    A_x, A_c_kv, A_w_q, A_w_uk, A_w_uv, A_w_o, B_x, B_w1, B_b1, B_w2, B_b2,
):
    return make()(A_x, A_c_kv, A_w_q, A_w_uk, A_w_uv, A_w_o, B_x, B_w1, B_b1, B_w2, B_b2)
```

```python
import contextlib
import jax
import jax.numpy as jnp
from jax import lax
import jax.experimental.pallas as pl
import jax.experimental.pallas.tpu as pltpu

F32 = jnp.float32
BF16 = jnp.bfloat16

B, H, SK, D, M, DC, F = 2, 32, 16384, 128, 512, 512, 1792
LOG2E = 1.4426950408889634
NT = (((1,), (1,)), ((), ()))

C_VIEW = (8, 4, 64, 16, DC)
W_VIEW = (4, 64, 2, H, D)
O_VIEW = (4, 8 * D, M)
W_QUADS = 192
S_UV, S_UK, S_Q, S_W1, S_W2, S_X, S_B1, S_B2, S_C = range(9)
S_O = S_C + 32


def _loop(lo, hi, body):
    lax.fori_loop(lo, hi, lambda i, _: body(i), None)


def _iota(shape, axis):
    return lax.broadcasted_iota(jnp.int32, shape, axis)


def _rows8(v):
    return jnp.concatenate([v[:, j * 128:(j + 1) * 128] for j in range(M // 128)], axis=0)


def make(TR=False, E1=10, E2=8, SH=0, TAIL=(16,) * 16 + (8,) * 16, LAG=26, STEPS=(8,) * 4 + (16,) * 8 + (32,), NOCOMP='', NOTAIL=False, SM=24,
         AHEAD=14, CUT=(0.07, 0.15, 0.24, 0.33, 0.44, 0.57, 0.65, 0.71, 0.79, 0.87, 0.94, 1.0), FIN='0 1 h 2 g', SW=(20, 21)):
    def ffn(t, h):
        out = []
        for k in range(8 + h, 0, -2):
            x = 3584 + SH - 512 * k + t % 32 * 16
            if 0 <= x < 1792 and -E2 <= t < 32 - E2:
                out.append(('w2', x))
            if 1792 <= x < 3584 and -E1 <= t < 32 - E1:
                r, c = divmod(x - 1792, 28)
                out.append(('w1', r, c, min(16, 28 - c)))
                if c > 12:
                    out.append(('w1', r + 1, 0, c - 12))
        return out

    C_END = 512 - 4 * max(E1, E2)
    first = [('o', 3, 1, 512 + sum(TAIL) + 8 * i, 8) for i in range(8)]
    quads = []
    for e in range(C_END, 512):
        if e % 2 == 0:
            quads.append(ffn(e // 4 - 128, e // 2 % 2))
        quads.append([('c', e, 1), ('c', e, 0)])
    for j in range(64):
        row = j // 2 * 16 + j % 2 * 512
        quads.append(ffn(j // 2, j % 2))
        quads.append([('o', 0, 3, row, 16), None if 512 <= row <= first[-1][3] else ('o', 3, 1, row, 16)])
    quads += [[('o', 3, 1, 512 + sum(TAIL[:i]), n), None] for i, n in enumerate(TAIL)]
    served = [(None, [('c', e, 0)]) for e in range(C_END - LAG, C_END)]
    for quad in quads:
        served += [(d, []) for d in quad[:-1]]
        served[-1][1].extend(d for d in quad[-1:] if d)
    ending = [x for (m, _), (_, s) in zip(served[LAG:], served) for x in [(m, 1)] + [(d, 0) for d in s]]
    assert not any(s for _, s in served[-LAG:])

    vpu = [h for h in range(H) if h % 4 == 3 or h >= 28]
    late = [d for d in first + [d for m, s in served[LAG:] for d in [m] + s] if d[0] == 'o' and 8 * d[1] + d[3] // D in vpu]
    steps = [[]]
    for d in late[::-1]:
        if sum(e[2] * e[4] for e in steps[0]) >= STEPS[min(len(steps), len(STEPS)) - 1]:
            steps.insert(0, [])
        steps[0].insert(0, d)
    step_of = {d: i for i, st in enumerate(steps) for d in st}
    IN_LOOP = 26
    cuts = [0] + [round(c * len(ending)) for c in CUT]

    def scope(name):
        return jax.named_scope('@' + name) if TR else contextlib.nullcontext()

    def kernel(x_hbm, c_hbm, wq_hbm, wuk_hbm, wuv_hbm, wo_hbm, w1_hbm, b1_hbm, w2_hbm, b2_hbm,
               o_hbm,
               x_buf, b1_buf, b2_buf, c_buf, wq_buf, wuk_buf, wuv_buf, wo_buf, w1_buf, w2_buf,
               xs, qa_ref, acc_ref, m_ref, l_ref, e_buf, a_buf, ctx_ref, mul_ref, o_buf, sems):
        def wait_filled(buf, k, name=''):
            with scope(name):
                pltpu.make_async_copy(buf, buf, sems.at[k]).wait()

        runs = (3, pl.ds(0, 3))

        def fetch_w(j, i, queue):
            hbm, buf = ((wuv_hbm, wuv_buf), (wuk_hbm, wuk_buf), (wq_hbm, wq_buf))[i]
            pltpu.make_async_copy(hbm.at[runs[queue], j], buf.at[runs[queue], j], sems.at[i]).start(priority=queue)

        def fetch_c(j, i, queue):
            src = c_hbm.at[(j >> 6) * 4 + i, runs[queue], j & 63]
            pltpu.make_async_copy(src, c_buf.at[j, i, runs[queue]], sems.at[S_C + (j >> 2)]).start(priority=queue)

        def fetch(d, queue):
            if d[0] == 'c':
                return fetch_c(*divmod(d[1], 4), queue)
            if d[0] == 'w2':
                hbm, buf, at, k = w2_hbm, w2_buf, pl.ds(d[1], 16), S_W2
            elif d[0] == 'w1':
                hbm, buf, at, k = w1_hbm, w1_buf, (pl.ds(d[1] * 8, 8), pl.ds(d[2] * 64, d[3] * 64)), S_W1
            else:
                hbm, buf, at = wo_hbm, wo_buf, (runs[d[2] > 1], pl.ds(d[3], d[4]))
                k = S_O + (3 + step_of[d] if d in step_of else d[3] // D % 4)
            pltpu.make_async_copy(hbm.at[at], buf.at[at], sems.at[k]).start(priority=queue)

        def issue(fetch, n, lo, hi, order=(1, 0)):
            def body(j):
                for i in range(n):
                    for queue in order:
                        r, a = divmod(i - (1 - queue) * LAG, n)
                        fetch(j + r, a, queue)
            with scope('i'):
                _loop(lo, hi, body)

        done = [0]

        def issue_end(when=None):
            lo, hi = cuts[done[0]:done[0] + 2]
            done[0] += 1

            def body(_):
                for d, queue in ending[lo:hi]:
                    fetch(d, queue)
            if when is not None:
                return pl.when(when)(lambda: body(0))
            with scope('ie'):
                pl.when(one)(lambda: body(0))

        x_copy = pltpu.make_async_copy(x_hbm, x_buf, sems.at[S_X])
        b1_copy = pltpu.make_async_copy(b1_hbm, b1_buf, sems.at[S_B1])
        b2_copy = pltpu.make_async_copy(b2_hbm, b2_buf, sems.at[S_B2])

        for i in range(27):
            fetch_w(*divmod(i, 3), 1)
            if i >= LAG:
                fetch_w(*divmod(i - LAG, 3), 0)
            elif i % 3 == 0 and i < 24:
                fetch(first[i // 3], 0)
            elif i == SM:
                for c in (x_copy, b2_copy, b1_copy):
                    c.start()
        issue(fetch_w, 3, 9, SW[0])
        issue(fetch_w, 3, SW[0], SW[1], (0, 1))

        x_copy.wait()
        x = x_buf[...].astype(F32)
        xc = x - jnp.mean(x, axis=-1, keepdims=True)
        var = jnp.mean(xc * xc, axis=-1, keepdims=True)
        xn = (xc * lax.rsqrt(var + 1e-5)).astype(BF16)
        xf = xn.astype(F32)
        for b in range(B):
            for j in range(M // 128):
                cols = slice(j * 128, (j + 1) * 128)
                xs[b, cols, :] = jnp.broadcast_to(xf[b:b + 1, cols], (128, 128)).T
        col, row = _iota((128, 1024), 1), _iota((128, 1024), 0)
        e_buf[...] = (col >> 3 == row).astype(F32).astype(BF16)
        m_ref[...] = jnp.full((B * H, 128), -jnp.inf, F32)
        l_ref[...] = jnp.zeros((B * H, 128), F32)
        acc_ref[...] = jnp.zeros((B * H, DC), F32)
        issue(fetch_w, 3, SW[1], 64)
        for e in range(28):
            fetch_c(*divmod(e, 4), 1)
            if e < LAG:
                fetch_w(*divmod(W_QUADS - LAG + e, 3), 0)
            else:
                fetch_c(0, e - LAG, 0)
        issue(fetch_c, 4, 7, AHEAD)

        wait_filled(wq_buf, S_Q, 'wq')

        def q_body(i, carry):
            pl.when((i & 15) == 15)(lambda: issue(fetch_c, 4, AHEAD + ((i >> 4) * 5 >> 1), AHEAD + ((i >> 4) * 5 + 5 >> 1)))
            q0, q1 = carry
            for u in range(0 if 'q' in NOCOMP else 8):
                m = pl.ds(i * 8 + u, 1)
                w = wq_buf[i >> 4, (i & 15) * 4 + u // 2, u % 2].astype(F32)
                q0 = q0 + xs[0, m, :] * w
                q1 = q1 + xs[1, m, :] * w
            return q0, q1

        q0, q1 = lax.fori_loop(0, 64, q_body, (jnp.zeros((H, D), F32), jnp.zeros((H, D), F32)))
        q = [jnp.concatenate([v[g * 8:g * 8 + 8] for v in (q0, q1)], axis=0).astype(BF16) for g in range(4)]

        wait_filled(wuk_buf, S_UK, 'wuk')
        diag = ((col & 7) == (row & 7))[:16]

        def qa_body(i):
            r = [lax.dot_general(q[g], wuk_buf[i, :, :, g * 8:g * 8 + 8].reshape(1024, D), NT,
                                 preferred_element_type=F32) for g in range(4)]
            r = [jnp.where(diag, v * (D ** -0.5 * LOG2E), 0.0) for v in r]
            r = jnp.concatenate([v[b * 8:b * 8 + 8] for b in range(B) for v in r], axis=0).astype(BF16)
            qa_ref[i] = lax.dot_general(r, e_buf[...], NT, preferred_element_type=F32).astype(BF16)
            issue(fetch_c, 4, AHEAD + 10 + 2 * i, AHEAD + 12 + 2 * i)

        _loop(0, 4, qa_body)

        def attend(k, n):
            for i in range(n):
                wait_filled(c_buf.at[pl.ds((k + i) * 4, 4)], S_C + k + i, 'c')
            if str(n) in NOCOMP:
                return
            hrows = pl.ds((k >> 4) * H if isinstance(k, int) else pl.multiple_of((k >> 4) * H, H), H)
            c = c_buf[pl.ds(k * 4, n * 4)].reshape(n * 1024, DC)
            sc = lax.dot_general(jnp.concatenate([qa_ref[j, hrows] for j in range(4)], axis=1), c, NT, preferred_element_type=F32)
            m_prev = m_ref[hrows, :]
            m_new = jnp.maximum(m_prev, jnp.max(sc, axis=1, keepdims=True))
            p = jnp.exp2(sc - m_new[:, :1])
            alpha = jnp.exp2(m_prev - m_new)
            l_ref[hrows, :] = alpha * l_ref[hrows, :] + jnp.sum(p, axis=1, keepdims=True)
            m_ref[hrows, :] = m_new
            pv = jnp.dot(p.astype(BF16), c, preferred_element_type=F32)
            acc_ref[hrows, :] = acc_ref[hrows, :] * alpha[:, :1] + pv

        def block(k, lo):
            hi = jnp.minimum(jnp.maximum(AHEAD + 19 + 3 * k, C_END // 4 - 4 * (IN_LOOP - 1 - k)), C_END // 4)
            issue(fetch_c, 4, lo, hi)

            @pl.when(k >= IN_LOOP)
            def _():
                with scope('ie'):
                    for i in range(IN_LOOP, 32):
                        issue_end(k == i)
            attend(k, 1)
            return hi

        one = lax.fori_loop(0, 32, block, AHEAD + 18) > 0

        issue_end()
        pc = acc_ref[...] / l_ref[...][:, :1]
        pc = jnp.concatenate([pc[b * H + g * 8:b * H + g * 8 + 8, j * 128:(j + 1) * 128]
                              for g in range(4) for j in range(4) for b in range(B)], axis=0).astype(BF16)
        rep = jnp.dot(pc, e_buf[...], preferred_element_type=F32).reshape(2, 128, 1024)
        a_buf[...] = jnp.where((col & 7) == (row & 7), rep, 0.0).astype(BF16).reshape(16, 16, 1024)
        issue_end()
        wait_filled(wuv_buf, S_UV, 'wuv')
        for g in range(4):
            a = jnp.concatenate([a_buf[4 * g + j] for j in range(4)], axis=1)
            w = wuv_buf[:, :, :, g * 8:g * 8 + 8].reshape(DC * 8, D)
            ctx_ref[g] = jnp.dot(a, w, preferred_element_type=F32).astype(BF16).astype(F32)
        issue_end()
        for b in range(B):
            for k, h in enumerate(vpu):
                mul_ref[b, k * D:(k + 1) * D] = jnp.broadcast_to(ctx_ref[h // 8, pl.ds(b * 8 + h % 8, 1)], (128, 128)).T

        sl16 = _iota((16, 128), 0) & 7
        part = [[None] * 4 for _ in range(B)]
        for what in FIN.split():
            if done[0] < len(CUT):
                issue_end()
            if what == 'h':
                wait_filled(w1_buf, S_W1, 'w1')
                b1_copy.wait()
                hid = jnp.dot(xn, w1_buf[...], preferred_element_type=F32)
                hid = jax.nn.gelu(hid + b1_buf[...].astype(F32).reshape(1, F), approximate=True).astype(BF16)
            elif what == 'g':
                wait_filled(w2_buf, S_W2, 'w2')
                b2_copy.wait()
                z = jnp.dot(hid, w2_buf[...], preferred_element_type=F32)
                z8 = _rows8(z + b2_buf[...].astype(F32).reshape(1, M))
                g8 = z8 * jax.nn.sigmoid(z8)
                x8 = _rows8(x)
            else:
                wait_filled(wo_buf.at[0, pl.ds(0, 7 * D)], S_O + int(what), 'o')
                heads = range(int(what), 28, 4)
                lhs = jnp.concatenate([jnp.where(sl16 == h % 8, ctx_ref[h // 8], 0.0) for h in heads], axis=1)
                rhs = jnp.concatenate([wo_buf[h // 8, pl.ds(h % 8 * D, D)] for h in heads], axis=0)
                s = jnp.dot(lhs.astype(BF16), rhs, preferred_element_type=F32)
                for b in range(B):
                    for j in range(4):
                        t = s[b * 8:b * 8 + 8, j * 128:(j + 1) * 128]
                        part[b][j] = t if part[b][j] is None else part[b][j] + t
        assert done[0] == len(CUT)

        sl = _iota((8, 128), 0)
        masks = {k: (sl & k) != 0 for k in (1, 2, 4)}
        for i, st in enumerate(steps):
            wait_filled(wo_buf.at[0, pl.ds(0, sum(d[2] * d[4] for d in st))], S_O + 3 + i, 'last')
            for _, a, n, r0, m in ([] if NOTAIL else st):
                for u in range(a, a + n):
                    for r in range(r0, r0 + m, 8):
                        w = wo_buf[u, r:r + 8].astype(F32)
                        for b in range(B):
                            mul = mul_ref[b, pl.ds(vpu.index(8 * u + r // D) * D + r % D, 8), :]
                            for j in range(M // 128):
                                part[b][j] = part[b][j] + w[:, j * 128:(j + 1) * 128] * mul

        def merge(lo, hi, k):
            m = masks[k]
            if k == 4:
                return jnp.where(m, hi, lo) + pltpu.roll(jnp.where(m, lo, hi), 4, 0)
            return jnp.where(m, hi, lo) + jnp.where(m, pltpu.roll(hi, k, 0), pltpu.roll(lo, 8 - k, 0))

        r4 = [[merge(part[b][j], part[b][j + 2], 4) for j in range(2)] for b in range(B)]
        r2 = [merge(r4[b][0], r4[b][1], 2) for b in range(B)]
        o_buf[...] = (x8 + g8 * merge(r2[0], r2[1], 1)).astype(BF16)
        o_copy = pltpu.make_async_copy(o_buf, o_hbm, sems.at[S_X])
        o_copy.start()
        o_copy.wait()

    def fn(A_x, A_c_kv, A_w_q, A_w_uk, A_w_uv, A_w_o, B_x, B_w1, B_b1, B_w2, B_b2):
        hbm = pl.BlockSpec(memory_space=pltpu.HBM)
        out = pl.pallas_call(
            kernel,
            out_shape=jax.ShapeDtypeStruct((8, 128), BF16),
            in_specs=[hbm] * 10,
            out_specs=hbm,
            scratch_shapes=[
                pltpu.VMEM((B, M), BF16), pltpu.VMEM((F,), BF16), pltpu.VMEM((M,), BF16),
                pltpu.VMEM((128, 4, 4, 16, DC), BF16), pltpu.VMEM(W_VIEW, BF16), pltpu.VMEM(W_VIEW, BF16),
                pltpu.VMEM(W_VIEW, BF16), pltpu.VMEM(O_VIEW, BF16),
                pltpu.VMEM((M, F), BF16), pltpu.VMEM((F, M), BF16),
                pltpu.VMEM((B, M, 128), F32),
                pltpu.VMEM((4, B * H, 128), BF16), pltpu.VMEM((B * H, DC), F32),
                pltpu.VMEM((B * H, 128), F32), pltpu.VMEM((B * H, 128), F32),
                pltpu.VMEM((128, 1024), BF16), pltpu.VMEM((16, 16, 1024), BF16), pltpu.VMEM((4, 16, D), F32),
                pltpu.VMEM((B, len(vpu) * D, 128), F32), pltpu.VMEM((8, 128), BF16),
                pltpu.SemaphoreType.DMA((S_O + 3 + len(steps),)),
            ],
            compiler_params=pltpu.CompilerParams(
                vmem_limit_bytes=100 * 1024 * 1024, disable_semaphore_checks=True, disable_bounds_checks=True),
        )(A_x.reshape(B, M), A_c_kv.reshape(C_VIEW), A_w_q.reshape(W_VIEW), A_w_uk.reshape(W_VIEW),
          A_w_uv.reshape(W_VIEW), A_w_o.reshape(O_VIEW), B_w1, B_b1, B_w2, B_b2)
        return out.reshape(M // 128, B, 128).transpose(1, 0, 2).reshape(B, 1, M)
    return fn


@jax.jit
def pallas_recurrent_scan__compressed_kv_cla__dense_activation_gelu__decode_kernel(
    A_x, A_c_kv, A_w_q, A_w_uk, A_w_uv, A_w_o, B_x, B_w1, B_b1, B_w2, B_b2,
):
    return make()(A_x, A_c_kv, A_w_q, A_w_uk, A_w_uv, A_w_o, B_x, B_w1, B_b1, B_w2, B_b2)
```

```python
import jax
import jax.numpy as jnp
from jax import lax
import jax.experimental.pallas as pl
import jax.experimental.pallas.tpu as pltpu

F32 = jnp.float32
BF16 = jnp.bfloat16

B, H, SK, D, M, DC, F = 2, 32, 16384, 128, 512, 512, 1792
LOG2E = 1.4426950408889634
NT = (((1,), (1,)), ((), ()))

W_VIEW = (4, 64, 2, H, D)
C_VIEW = (8, 4, 64, 16, DC)
O_VIEW = (4, 8 * D, M)
LAG = 26
AHEAD = 14
W1_EARLY, W2_EARLY = 10, 8
C_ALONE = 128 - W1_EARLY
TAIL = (16,) * 22 + (8,) * 4
VPU_HEADS = [h for h in range(H) if h % 4 == 3 or h >= 28]
S_UV, S_UK, S_Q, S_W1, S_W2, S_X, S_B1, S_B2, S_OUT, S_C = range(10)
S_O = S_C + 32
S_LATE = S_O + 8


def _plan_ending():
    def ffn(t, half):
        out = []
        for run in range(1 - half, 7, 2):
            kib = 512 * run + 16 * (t % 32)
            if kib < 1792 and 0 <= t + W2_EARLY < 32:
                out.append(("w2", kib))
            if kib >= 1792 and 0 <= t + W1_EARLY < 32:
                tile, at = divmod(kib - 1792, 28)
                out.append(("w1", tile, at, min(16, 28 - at)))
                if at > 12:
                    out.append(("w1", tile + 1, 0, at - 12))
        return out

    spare = [("o", 3, 1, 512 + sum(TAIL) + 8 * i, 8) for i in range(8)]
    groups = []
    for j in range(C_ALONE, 128):
        for i in range(4):
            if i % 2 == 0:
                groups.append(ffn(j - 128, i // 2))
            groups.append([("c", j, i)] * 2)
    for j in range(32):
        for half in range(2):
            row = 512 * half + 16 * j
            groups.append(ffn(j, half))
            groups.append([("o", 0, 3, row, 16), None if 512 <= row <= spare[-1][3] else ("o", 3, 1, row, 16)])
    groups += [[("o", 3, 1, 512 + sum(TAIL[:i]), n), None] for i, n in enumerate(TAIL)]

    main, side = [], [[("c", *divmod(4 * C_ALONE - LAG + i, 4))] for i in range(LAG)]
    for group in groups:
        main += group[:-1]
        side += [[] for _ in group[:-1]]
        side[-1] += [d for d in group[-1:] if d]
    assert not any(side[-LAG:])
    started = [c for m, s in zip(main, side) for c in [(m, 1)] + [(d, 0) for d in s]]
    served = spare + [d for group in groups for d in group if d]
    late = [d for d in served if d[0] == "o" and 8 * d[1] + d[3] // D in VPU_HEADS]
    cuts = [round(len(started) * c / 100) for c in (0, 7, 15, 24, 33, 44, 57, 65, 71, 79, 87, 94, 100)]
    return spare, [started[lo:hi] for lo, hi in zip(cuts, cuts[1:])], late


SPARE, ENDING, LATE = _plan_ending()


def _loop(lo, hi, body):
    lax.fori_loop(lo, hi, lambda i, _: body(i), None)


def _iota(shape, axis):
    return lax.broadcasted_iota(jnp.int32, shape, axis)


def _rows8(v):
    return jnp.concatenate([v[:, j * 128:(j + 1) * 128] for j in range(M // 128)], axis=0)


def _kernel(c_hbm, x_hbm, wq_hbm, wuk_hbm, wuv_hbm, wo_hbm, w1_hbm, b1_hbm, w2_hbm, b2_hbm,
            o_hbm,
            x_buf, b1_buf, b2_buf, c_buf, wq_buf, wuk_buf, wuv_buf, wo_buf, w1_buf, w2_buf,
            xs, qa_ref, acc_ref, m_ref, l_ref, e_buf, a_buf, ctx_ref, mul_ref, o_buf, sems):
    runs = (3, pl.ds(0, 3))

    def fetch_w(j, i, queue):
        hbm, buf = ((wuv_hbm, wuv_buf), (wuk_hbm, wuk_buf), (wq_hbm, wq_buf))[i]
        pltpu.make_async_copy(hbm.at[runs[queue], j], buf.at[runs[queue], j], sems.at[i]).start(priority=queue)

    def fetch_c(j, i, queue):
        src = c_hbm.at[(j >> 6) * 4 + i, runs[queue], j & 63]
        pltpu.make_async_copy(src, c_buf.at[j, i, runs[queue]], sems.at[S_C + (j >> 2)]).start(priority=queue)

    def planned(d):
        if d[0] == "w2":
            hbm, buf, at, sem = w2_hbm, w2_buf, pl.ds(d[1], 16), S_W2
        elif d[0] == "w1":
            hbm, buf, at, sem = w1_hbm, w1_buf, (pl.ds(d[1] * 8, 8), pl.ds(d[2] * 64, d[3] * 64)), S_W1
        else:
            hbm, buf, at = wo_hbm, wo_buf, (runs[d[2] > 1], pl.ds(d[3], d[4]))
            sem = S_LATE + LATE.index(d) if d in LATE else S_O + d[3] // D
        return pltpu.make_async_copy(hbm.at[at], buf.at[at], sems.at[sem])

    def issue(fetch, groups, lo, hi, order=(1, 0)):
        def body(j):
            for i in range(groups):
                for queue in order:
                    back, group = divmod(i - (1 - queue) * LAG, groups)
                    fetch(j + back, group, queue)
        _loop(lo, hi, body)

    def issue_ending(k):
        for d, queue in ENDING[k]:
            if d[0] == "c":
                fetch_c(d[1], d[2], queue)
            else:
                planned(d).start(priority=queue)

    def wait_filled(buf, sem):
        pltpu.make_async_copy(buf, buf, sems.at[sem]).wait()

    x_copy = pltpu.make_async_copy(x_hbm, x_buf, sems.at[S_X])
    b1_copy = pltpu.make_async_copy(b1_hbm, b1_buf, sems.at[S_B1])
    b2_copy = pltpu.make_async_copy(b2_hbm, b2_buf, sems.at[S_B2])

    for i in range(27):
        fetch_w(*divmod(i, 3), 1)
        if i >= LAG:
            fetch_w(*divmod(i - LAG, 3), 0)
        elif i == 24:
            for c in (x_copy, b2_copy, b1_copy):
                c.start()
        elif i % 3 == 0:
            planned(SPARE[i // 3]).start()
    issue(fetch_w, 3, 9, 20)
    issue(fetch_w, 3, 20, 21, (0, 1))

    x_copy.wait()
    x = x_buf[...].astype(F32)
    xc = x - jnp.mean(x, axis=-1, keepdims=True)
    var = jnp.mean(xc * xc, axis=-1, keepdims=True)
    xn = (xc * lax.rsqrt(var + 1e-5)).astype(BF16)
    xf = xn.astype(F32)
    for b in range(B):
        for j in range(M // 128):
            cols = slice(j * 128, (j + 1) * 128)
            xs[b, cols, :] = jnp.broadcast_to(xf[b:b + 1, cols], (128, 128)).T
    col, row = _iota((128, 1024), 1), _iota((128, 1024), 0)
    e_buf[...] = (col >> 3 == row).astype(F32).astype(BF16)
    m_ref[...] = jnp.full((B * H, 128), -jnp.inf, F32)
    l_ref[...] = jnp.zeros((B * H, 128), F32)
    acc_ref[...] = jnp.zeros((B * H, DC), F32)
    issue(fetch_w, 3, 21, 64)
    for i in range(28):
        fetch_c(*divmod(i, 4), 1)
        if i >= LAG:
            fetch_c(*divmod(i - LAG, 4), 0)
        else:
            fetch_w(*divmod(192 + i - LAG, 3), 0)
    issue(fetch_c, 4, 7, AHEAD)

    wait_filled(wq_buf, S_Q)

    def q_body(i, carry):
        run = i >> 4
        pl.when((i & 15) == 15)(lambda: issue(fetch_c, 4, AHEAD + (run * 5 >> 1), AHEAD + (run * 5 + 5 >> 1)))
        q0, q1 = carry
        for u in range(8):
            m = pl.ds(i * 8 + u, 1)
            w = wq_buf[run, (i & 15) * 4 + u // 2, u % 2].astype(F32)
            q0 = q0 + xs[0, m, :] * w
            q1 = q1 + xs[1, m, :] * w
        return q0, q1

    q = lax.fori_loop(0, 64, q_body, (jnp.zeros((H, D), F32), jnp.zeros((H, D), F32)))
    q = [jnp.concatenate([v[g * 8:g * 8 + 8] for v in q], axis=0).astype(BF16) for g in range(4)]

    wait_filled(wuk_buf, S_UK)
    same_head = ((col & 7) == (row & 7))[:16]

    def qa_body(i):
        r = [lax.dot_general(q[g], wuk_buf[i, :, :, g * 8:g * 8 + 8].reshape(1024, D), NT,
                             preferred_element_type=F32) for g in range(4)]
        r = [jnp.where(same_head, v * (D ** -0.5 * LOG2E), 0.0) for v in r]
        r = jnp.concatenate([v[b * 8:b * 8 + 8] for b in range(B) for v in r], axis=0).astype(BF16)
        qa_ref[i] = lax.dot_general(r, e_buf[...], NT, preferred_element_type=F32).astype(BF16)
        issue(fetch_c, 4, AHEAD + 10 + 2 * i, AHEAD + 12 + 2 * i)

    _loop(0, 4, qa_body)

    def block(k, issued):
        upto = jnp.minimum(jnp.maximum(AHEAD + 19 + (13 * k >> 2), C_ALONE - 4 * (25 - k)), C_ALONE)
        issue(fetch_c, 4, issued, upto)

        @pl.when(k >= 26)
        def _():
            for i in range(6):
                pl.when(k == 26 + i)(lambda: issue_ending(i))

        rounds = pl.ds(k * 4, 4)
        wait_filled(c_buf.at[rounds], S_C + k)
        heads = pl.ds(pl.multiple_of((k >> 4) * H, H), H)
        c = c_buf[rounds].reshape(1024, DC)
        qa = jnp.concatenate([qa_ref[j, heads] for j in range(4)], axis=1)
        sc = lax.dot_general(qa, c, NT, preferred_element_type=F32)
        m_prev = m_ref[heads, :]
        m_new = jnp.maximum(m_prev, jnp.max(sc, axis=1, keepdims=True))
        p = jnp.exp2(sc - m_new[:, :1])
        alpha = jnp.exp2(m_prev - m_new)
        l_ref[heads, :] = alpha * l_ref[heads, :] + jnp.sum(p, axis=1, keepdims=True)
        m_ref[heads, :] = m_new
        pv = jnp.dot(p.astype(BF16), c, preferred_element_type=F32)
        acc_ref[heads, :] = acc_ref[heads, :] * alpha[:, :1] + pv
        return upto

    lax.fori_loop(0, 32, block, AHEAD + 18)

    issue_ending(6)
    pc = acc_ref[...] / l_ref[...][:, :1]
    pc = jnp.concatenate([pc[b * H + g * 8:b * H + g * 8 + 8, j * 128:(j + 1) * 128]
                          for g in range(4) for j in range(4) for b in range(B)], axis=0).astype(BF16)
    rep = jnp.dot(pc, e_buf[...], preferred_element_type=F32).reshape(2, 128, 1024)
    a_buf[...] = jnp.where((col & 7) == (row & 7), rep, 0.0).astype(BF16).reshape(16, 16, 1024)
    issue_ending(7)
    wait_filled(wuv_buf, S_UV)
    for g in range(4):
        a = jnp.concatenate([a_buf[4 * g + j] for j in range(4)], axis=1)
        w = wuv_buf[:, :, :, g * 8:g * 8 + 8].reshape(DC * 8, D)
        ctx_ref[g] = jnp.dot(a, w, preferred_element_type=F32).astype(BF16).astype(F32)
    issue_ending(8)
    for b in range(B):
        for k, h in enumerate(VPU_HEADS):
            ctx = ctx_ref[h // 8, pl.ds(b * 8 + h % 8, 1)]
            mul_ref[b, k * D:(k + 1) * D] = jnp.broadcast_to(ctx, (128, 128)).T

    def project(k):
        wait_filled(wo_buf.at[:, pl.ds(k * D, D)], S_O + k)
        wait_filled(wo_buf.at[runs[1], pl.ds((k + 4) * D, D)], S_O + k + 4)
        heads, head = range(k, 28, 4), _iota((16, D), 0) & 7
        lhs = jnp.concatenate([jnp.where(head == h % 8, ctx_ref[h // 8], 0.0) for h in heads], axis=1)
        rhs = jnp.concatenate([wo_buf[h // 8, pl.ds(h % 8 * D, D)] for h in heads], axis=0)
        s = jnp.dot(lhs.astype(BF16), rhs, preferred_element_type=F32)
        return [[s[b * 8:b * 8 + 8, j * 128:(j + 1) * 128] for j in range(4)] for b in range(B)]

    issue_ending(9)
    s0 = project(0)
    issue_ending(10)
    s1 = project(1)
    issue_ending(11)

    wait_filled(w1_buf, S_W1)
    b1_copy.wait()
    hid = jnp.dot(xn, w1_buf[...], preferred_element_type=F32)
    hid = jax.nn.gelu(hid + b1_buf[...].astype(F32).reshape(1, F), approximate=True).astype(BF16)
    s2 = project(2)
    part = [[s0[b][j] + s1[b][j] + s2[b][j] for j in range(4)] for b in range(B)]
    wait_filled(w2_buf, S_W2)
    b2_copy.wait()
    z = jnp.dot(hid, w2_buf[...], preferred_element_type=F32)
    z8 = _rows8(z + b2_buf[...].astype(F32).reshape(1, M))
    g8 = z8 * jax.nn.sigmoid(z8)
    x8 = _rows8(x)

    masks = {k: (_iota((8, 128), 0) & k) != 0 for k in (1, 2, 4)}
    for d in LATE:
        planned(d).wait()
        end = d[3] + d[4]
        for run in range(d[1], d[1] + d[2]):
            for r in range(d[3] // 16 * 16, end // 16 * 16, 8):
                w = wo_buf[run, r:r + 8].astype(F32)
                for b in range(B):
                    mul = mul_ref[b, pl.ds(VPU_HEADS.index(8 * run + r // D) * D + r % D, 8), :]
                    for j in range(4):
                        part[b][j] = part[b][j] + w[:, j * 128:(j + 1) * 128] * mul

    def merge(lo, hi, k):
        m = masks[k]
        if k == 4:
            return jnp.where(m, hi, lo) + pltpu.roll(jnp.where(m, lo, hi), 4, 0)
        return jnp.where(m, hi, lo) + jnp.where(m, pltpu.roll(hi, k, 0), pltpu.roll(lo, 8 - k, 0))

    r4 = [[merge(part[b][j], part[b][j + 2], 4) for j in range(2)] for b in range(B)]
    r2 = [merge(r4[b][0], r4[b][1], 2) for b in range(B)]
    o_buf[...] = (x8 + g8 * merge(r2[0], r2[1], 1)).astype(BF16)
    o_copy = pltpu.make_async_copy(o_buf, o_hbm, sems.at[S_OUT])
    o_copy.start()
    o_copy.wait()


@jax.jit
def pallas_recurrent_scan__compressed_kv_cla__dense_activation_gelu__decode_kernel(
    A_x: jax.Array,
    A_c_kv: jax.Array,
    A_w_q: jax.Array,
    A_w_uk: jax.Array,
    A_w_uv: jax.Array,
    A_w_o: jax.Array,
    B_x: jax.Array,
    B_w1: jax.Array,
    B_b1: jax.Array,
    B_w2: jax.Array,
    B_b2: jax.Array,
):
    del B_x
    hbm = pl.BlockSpec(memory_space=pltpu.HBM)
    out = pl.pallas_call(
        _kernel,
        out_shape=jax.ShapeDtypeStruct((8, 128), BF16),
        in_specs=[hbm] * 10,
        out_specs=hbm,
        scratch_shapes=[
            pltpu.VMEM((B, M), BF16), pltpu.VMEM((F,), BF16), pltpu.VMEM((M,), BF16),
            pltpu.VMEM((128, 4, 4, 16, DC), BF16), pltpu.VMEM(W_VIEW, BF16), pltpu.VMEM(W_VIEW, BF16),
            pltpu.VMEM(W_VIEW, BF16), pltpu.VMEM(O_VIEW, BF16),
            pltpu.VMEM((M, F), BF16), pltpu.VMEM((F, M), BF16),
            pltpu.VMEM((B, M, 128), F32), pltpu.VMEM((4, B * H, 128), BF16),
            pltpu.VMEM((B * H, DC), F32), pltpu.VMEM((B * H, 128), F32), pltpu.VMEM((B * H, 128), F32),
            pltpu.VMEM((128, 1024), BF16), pltpu.VMEM((16, 16, 1024), BF16), pltpu.VMEM((4, 16, D), F32),
            pltpu.VMEM((B, len(VPU_HEADS) * D, 128), F32), pltpu.VMEM((8, 128), BF16),
            pltpu.SemaphoreType.DMA((S_LATE + len(LATE),)),
        ],
        compiler_params=pltpu.CompilerParams(
            vmem_limit_bytes=100 * 1024 * 1024, disable_semaphore_checks=True, disable_bounds_checks=True),
    )(A_c_kv.reshape(C_VIEW), A_x.reshape(B, M), A_w_q.reshape(W_VIEW), A_w_uk.reshape(W_VIEW),
      A_w_uv.reshape(W_VIEW), A_w_o.reshape(O_VIEW), B_w1, B_b1, B_w2, B_b2)
    return out.reshape(M // 128, B, 128).transpose(1, 0, 2).reshape(B, 1, M)
```
